```python
import os as _os
_os.environ.setdefault("JAX_PLATFORMS", "cpu")
import jax
import jax.numpy as jnp

def _softmax(x, axis=-1):
    return jax.nn.softmax(x, axis=axis)
def _gelu(x):
    return jax.nn.gelu(x, approximate=True)
def _silu(x):
    return jax.nn.silu(x)
def _sigmoid(x):
    return jax.nn.sigmoid(x)
def _layernorm(x, axis=-1, eps=1e-5):
    m = jnp.mean(x, axis=axis, keepdims=True)
    v = jnp.var(x, axis=axis, keepdims=True)
    return (x - m) / jnp.sqrt(v + eps)
def _scatter_add(tgt, idx, src, axis=0):
    return tgt.at[idx].add(src)
def _segment_sum(src, seg, n):
    return jax.ops.segment_sum(src, seg, n)
class _Rng:
    def __init__(self, key):
        self._k = key
    def _next(self):
        self._k, sub = jax.random.split(self._k)
        return sub
    def normal(self, shape):
        return jax.random.normal(self._next(), shape, dtype=jnp.bfloat16)
    def randint(self, lo, hi, shape):
        return jax.random.randint(self._next(), shape, lo, hi, dtype=jnp.int32)
    def uniform(self, shape, lo=0.0, hi=1.0):
        return jax.random.uniform(self._next(), shape, jnp.bfloat16, lo, hi)
    def permutation(self, n):
        return jax.random.permutation(self._next(), n)


kernel_name = 'concat_heads__gqa_block_cached__gqa_block_cached__decode'

def setup_inputs():
    _rng = _Rng(jax.random.key(int.from_bytes(__import__("os").urandom(4), "little")))
    _w = (lambda a: (lambda t: t.astype(jnp.bfloat16) if jnp.issubdtype(t.dtype, jnp.floating) else t)(jnp.asarray(a)))
    def _A_setup():
        B, Sq, D = 2, 1, 576
        Hq, Hkv, Sk, Dh = 32, 16, 4096, 128
        assert Hq % Hkv == 0, (Hq, Hkv)
        return {
            "x": _w((lambda *s: _rng.normal(s) * 0.8)(B, Sq, D)),
            "k_cache": _w((lambda *s: _rng.normal(s) * 0.8)(B, Hkv, Sk, Dh)),
            "v_cache": _w((lambda *s: _rng.normal(s) * 0.05)(B, Hkv, Sk, Dh)),
            "wq": _w((lambda *s: _rng.normal(s) * 0.8)(D, Hq * Dh) * (D ** -0.5)),
            "wo": _w((lambda *s: _rng.normal(s) * 0.05)(Hq * Dh, D) * ((Hq * Dh) ** -0.5)),
        }
    _A_in = _A_setup()

    def _B_setup():
        B, Sq, D = 2, 1, 576
        Hq, Hkv, Sk, Dh = 32, 16, 4096, 128
        assert Hq % Hkv == 0, (Hq, Hkv)
        return {
            "x": _w((lambda *s: _rng.normal(s) * 0.8)(B, Sq, D)),
            "k_cache": _w((lambda *s: _rng.normal(s) * 0.8)(B, Hkv, Sk, Dh)),
            "v_cache": _w((lambda *s: _rng.normal(s) * 0.05)(B, Hkv, Sk, Dh)),
            "wq": _w((lambda *s: _rng.normal(s) * 0.8)(D, Hq * Dh) * (D ** -0.5)),
            "wo": _w((lambda *s: _rng.normal(s) * 0.05)(Hq * Dh, D) * ((Hq * Dh) ** -0.5)),
        }
    _B_in = _B_setup()

    return {
        "A_x": _A_in["x"],
        "A_k_cache": _A_in["k_cache"],
        "A_v_cache": _A_in["v_cache"],
        "A_wq": _A_in["wq"],
        "A_wo": _A_in["wo"],
        "B_x": _B_in["x"],
        "B_k_cache": _B_in["k_cache"],
        "B_v_cache": _B_in["v_cache"],
        "B_wq": _B_in["wq"],
        "B_wo": _B_in["wo"],
    }

def reference(A_x, A_k_cache, A_v_cache, A_wq, A_wo, B_x, B_k_cache, B_v_cache, B_wq, B_wo):
    def _A_ref(x, k_cache, v_cache, wq, wo):
        B, Sq, D = x.shape
        Hq, Dh = 32, 128
        Hkv = k_cache.shape[1]
        rep = Hq // Hkv
        q = (lambda x, *d: x.transpose(*d))((x @ wq).reshape(B, Sq, Hq, Dh), 0, 2, 1, 3)
        k = jnp.repeat(k_cache, rep, axis=1)
        v = jnp.repeat(v_cache, rep, axis=1)
        scores = jnp.einsum("bhqd,bhkd->bhqk", q, k) * (Dh ** -0.5)
        p = _softmax(scores, axis=-1)
        o = jnp.einsum("bhqk,bhkd->bhqd", p, v)
        return (lambda x, *d: x.transpose(*d))(o, 0, 2, 1, 3).reshape(B, Sq, Hq * Dh) @ wo

    def _B_ref(x, k_cache, v_cache, wq, wo):
        B, Sq, D = x.shape
        Hq, Dh = 32, 128
        Hkv = k_cache.shape[1]
        rep = Hq // Hkv
        q = (lambda x, *d: x.transpose(*d))((x @ wq).reshape(B, Sq, Hq, Dh), 0, 2, 1, 3)
        k = jnp.repeat(k_cache, rep, axis=1)
        v = jnp.repeat(v_cache, rep, axis=1)
        scores = jnp.einsum("bhqd,bhkd->bhqk", q, k) * (Dh ** -0.5)
        p = _softmax(scores, axis=-1)
        o = jnp.einsum("bhqk,bhkd->bhqd", p, v)
        return (lambda x, *d: x.transpose(*d))(o, 0, 2, 1, 3).reshape(B, Sq, Hq * Dh) @ wo

    a = _A_ref(A_x, A_k_cache, A_v_cache, A_wq, A_wo)
    b = _B_ref(B_x, B_k_cache, B_v_cache, B_wq, B_wo)
    return jnp.concatenate([a, b], axis=-1)
```

```python
import math

import jax
import jax.numpy as jnp
from jax import lax
import jax.experimental.pallas as pl
import jax.experimental.pallas.tpu as pltpu

_NT = (((1,), (1,)), ((), ()))


def make(piece=128, nc=4, depth=3, wr=16, wc=1024, nobc=False, qsteps=8, tail=1, unroll=False, outdma=False):
    B, D, HQ, HKV, SK, DH = 2, 576, 32, 16, 4096, 128
    E = HQ * DH
    NH = B * HKV
    CH = SK // nc
    NS = 2 * nc
    RS = SK // NS
    C2 = (DH ** -0.5) * math.log2(math.e)
    LOOK = depth - 1
    f32, bf16 = jnp.float32, jnp.bfloat16

    def kernel(ax, ak, av, aq, ao, bx, bk, bv, bq, bo, o_ref,
               xbuf, wqbuf, wobuf, kvbuf, qbuf, obuf, sbuf, xsem, wqsem, wosem, kvsem, osem, outbuf):
        row = lax.broadcasted_iota(jnp.int32, (8, DH), 0)

        def w_issue(src, r0, dst, d0, sem):
            for t in range(E // wc):
                cs = pl.ds(t * wc, wc)
                pltpu.make_async_copy(src.at[pl.ds(r0, wr), cs], dst.at[pl.ds(d0, wr), cs], sem).start(priority=t % 2)

        def kv_issue(k, v, j, slot, step):
            for t in range(RS // piece):
                off = pl.multiple_of(step * RS + t * piece, piece)
                src = pl.ds(pl.multiple_of(j * SK + off, piece), piece)
                for w, ref in enumerate((k, v)):
                    pltpu.make_async_copy(ref.at[src], kvbuf.at[slot, w, pl.ds(off, piece)], kvsem.at[slot]).start(priority=w)

        NWU = D // wr

        def wo_issue(u):
            d0 = pl.multiple_of(u * wr, wr)
            sem = wosem.at[d0 // 128]

            @pl.when(u < NWU)
            def _():
                w_issue(ao, d0, wobuf, d0, sem)

            @pl.when((u >= NWU) & (u < 2 * NWU))
            def _():
                w_issue(bo, pl.multiple_of(d0 - D, wr), wobuf, d0, sem)

        UPS = (RS * 2 * DH) // (wr * E)

        def issue(j, step):
            slot = j % depth

            @pl.when(j < NH)
            def _():
                kv_issue(ak, av, j, slot, step)

            @pl.when((j >= NH) & (j < 2 * NH))
            def _():
                kv_issue(bk, bv, j - NH, slot, step)

            @pl.when(j >= 2 * NH)
            def _():
                for t in range(UPS):
                    wo_issue(((j - 2 * NH) * NS + step) * UPS + t)

        xcp = [pltpu.make_async_copy(s, xbuf.at[i], xsem.at[i]) for i, s in enumerate((ax, bx))]
        for i, src in enumerate((aq, bq)):
            @pl.loop(0, NWU)
            def _(u):
                r0 = pl.multiple_of(u * wr, wr)
                w_issue(src, r0, wqbuf.at[i], r0, wqsem.at[i])
            if i == 0:
                xcp[0].start()
                xcp[1].start(priority=1)
        xcp[0].wait()
        xcp[1].wait()

        QW = E // qsteps
        xrow = lax.broadcasted_iota(jnp.int32, (8, D), 0)

        @pl.loop(0, 2)
        def _(br):
            pltpu.make_async_copy(wqbuf.at[br], wqbuf.at[br], wqsem.at[br]).wait()
            x = xbuf[br].astype(f32)
            x8 = jnp.where(xrow % 2 == 0, x[0:1], x[1:2]).astype(bf16)

            @pl.loop(0, qsteps)
            def _(c):
                for t in range(NS // qsteps):
                    kv_issue(ak, av, br, br, c * (NS // qsteps) + t)
                w = wqbuf[br, :, pl.ds(pl.multiple_of(c * QW, QW), QW)]
                q = jnp.dot(x8, w, preferred_element_type=f32)
                for t in range(QW // (2 * DH)):
                    q0 = q[:, 2 * t * DH:(2 * t + 1) * DH]
                    q1 = q[:, (2 * t + 1) * DH:(2 * t + 2) * DH]
                    qbuf[br * HKV + c * (QW // (2 * DH)) + t] = jnp.where(row % 4 < 2, q0, q1)

        for j in range(2, LOOK):
            @pl.loop(0, NS)
            def _(c):
                kv_issue(ak, av, j, j, c)

        @pl.loop(0, 2 * NH)
        def _(i):
            slot = i % depth
            pltpu.make_async_copy(kvbuf.at[slot], kvbuf.at[slot], kvsem.at[slot]).wait()
            q = qbuf[(i // NH) * HKV + i % HKV].astype(bf16)

            def qk(c, m):
                issue(i + LOOK, c)
                k = kvbuf[slot, 0, pl.ds(pl.multiple_of(c * CH, CH), CH), :]
                s = lax.dot_general(q, k, _NT, preferred_element_type=f32)
                sbuf[c] = s
                for t in range(CH // DH):
                    m = jnp.maximum(m, s[:, t * DH:(t + 1) * DH])
                return m

            m = lax.fori_loop(0, nc, qk, jnp.full((8, DH), -jnp.inf, f32), unroll=unroll)
            m = jnp.max(m, axis=1, keepdims=True)

            def pv(c, carry):
                l, acc = carry
                issue(i + LOOK, nc + c)
                p = jnp.exp2((sbuf[c] - m) * C2)
                for t in range(CH // DH):
                    l = l + p[:, t * DH:(t + 1) * DH]
                v = kvbuf[slot, 1, pl.ds(pl.multiple_of(c * CH, CH), CH), :]
                return l, acc + jnp.dot(p.astype(bf16), v, preferred_element_type=f32)

            z = jnp.zeros((8, DH), f32)
            l, acc = lax.fori_loop(0, nc, pv, (z, z), unroll=unroll)
            obuf[i] = acc / jnp.sum(l, axis=1, keepdims=True)

        cols = []
        for h in range(HKV):
            oa = jnp.where(row % 2 == 0, obuf[h], obuf[HKV + h])
            ob = jnp.where(row % 2 == 0, obuf[NH + h], obuf[NH + HKV + h])
            o = jnp.where(row < 4, oa, ob)
            cols.append(jnp.where(row % 4 < 2, o, 0.0))
            cols.append(jnp.where(row % 4 < 2, 0.0, o))
        o_all = jnp.concatenate(cols, axis=1).astype(bf16)

        DONE = LOOK * NS * UPS
        UPT = 128 // wr
        lane = lax.broadcasted_iota(jnp.int32, (2, DH), 1)

        @pl.loop(0, 2 * D // 128)
        def _(t):
            @pl.loop(0, UPT)
            def _(u):
                wo_issue(DONE + t * UPT + u)
            rows = pl.ds(pl.multiple_of(t * 128, 128), 128)
            pltpu.make_async_copy(wobuf.at[rows], wobuf.at[rows], wosem.at[t]).wait()
            r = lax.dot_general(o_all, wobuf[rows, :], _NT, preferred_element_type=f32)
            res = jnp.where(lane + t * 128 < D, r[0:2] + r[2:4], r[4:6] + r[6:8])
            (outbuf if outdma else o_ref)[:, rows] = res.astype(bf16)

        if outdma:
            cp = pltpu.make_async_copy(outbuf, o_ref, osem)
            cp.start()
            cp.wait()

    @jax.jit
    def fn(A_x, A_k_cache, A_v_cache, A_wq, A_wo, B_x, B_k_cache, B_v_cache, B_wq, B_wo):
        rows = lambda t: t.reshape(-1, DH)
        hbm = pl.BlockSpec(memory_space=pltpu.HBM)
        dma = pltpu.SemaphoreType.DMA
        out = pl.pallas_call(
            kernel,
            out_shape=jax.ShapeDtypeStruct((B, 2 * D), bf16),
            in_specs=[hbm] * 10,
            out_specs=hbm if outdma else pl.BlockSpec(memory_space=pltpu.VMEM),
            scratch_shapes=[
                pltpu.VMEM((2, B, D), bf16),
                pltpu.VMEM((2, D, E), bf16),
                pltpu.VMEM((2 * D, E), bf16),
                pltpu.VMEM((depth, 2, SK, DH), bf16),
                pltpu.VMEM((2 * HKV, 8, DH), f32),
                pltpu.VMEM((2 * NH, 8, DH), f32),
                pltpu.VMEM((nc, 8, CH), f32),
                dma((2,)), dma((2,)), dma((2 * D // 128,)), dma((depth,)), dma(()),
                pltpu.VMEM((B, 2 * D), bf16),
            ],
            compiler_params=pltpu.CompilerParams(vmem_limit_bytes=64 * 2**20, disable_bounds_checks=nobc),
        )(A_x.reshape(B, D), rows(A_k_cache), rows(A_v_cache), A_wq, A_wo.T,
          B_x.reshape(B, D), rows(B_k_cache), rows(B_v_cache), B_wq, B_wo.T)
        return out.reshape(B, 1, 2 * D)

    return fn


_fn = make(piece=64, nc=2, qsteps=4, unroll=True, nobc=True)


@jax.jit
def pallas_concat_heads__gqa_block_cached__gqa_block_cached__decode_kernel(
        A_x, A_k_cache, A_v_cache, A_wq, A_wo, B_x, B_k_cache, B_v_cache, B_wq, B_wo):
    return _fn(A_x, A_k_cache, A_v_cache, A_wq, A_wo, B_x, B_k_cache, B_v_cache, B_wq, B_wo)
```

```python
import math

import jax
import jax.numpy as jnp
from jax import lax
import jax.experimental.pallas as pl
import jax.experimental.pallas.tpu as pltpu

_NT = (((1,), (1,)), ((), ()))


def make(vx=1, wq_parts=4, wo_parts=4, pre=4, lastsplit=False, lead=2, boost=2, skip=0, xpos=1, outdma=False,
         small=True, order=0, nobc=True, eper=1):
    B, D, HQ, HKV, SK, DH = 2, 576, 32, 16, 4096, 128
    E = HQ * DH
    NH = B * HKV
    GH, NSLOT, PIECE = 8, 3, 128
    NSTEP = 4 * NH
    C2 = (DH ** -0.5) * math.log2(math.e)
    NT = 2 * D // 128
    ER = 256
    MR = D - ER
    NU = MR // 8 // wo_parts
    HK = E // 2
    NES = 16
    f32, bf16 = jnp.float32, jnp.bfloat16

    def ds(start, size, align):
        return pl.ds(pl.multiple_of(start, align), size)

    def kernel(ax, ak, av, aq, ao, bx, bk, bv, bq, bo, o_ref,
               xbuf, wqbuf, wobuf, kvbuf, qbuf, sbuf, obuf, oall, accbuf, outbuf, xsem, wqsem, wosem, kvsem, esem, osem):
        row = lax.broadcasted_iota(jnp.int32, (8, DH), 0)

        def start(src, dst, sem, queue):
            pltpu.make_async_copy(src, dst, sem).start(priority=queue)

        def wait(buf, sem):
            pltpu.make_async_copy(buf, buf, sem).wait()

        def kv_step(k, v, g, slot, h0, nh, r, sem):
            npc = 16 // nh
            for t in range(npc):
                for hi in range(nh):
                    h = hi if order == 0 else int(format(hi, '0%db' % (nh.bit_length() - 1))[::-1], 2)
                    for w, ref in enumerate((k, v)):
                        off = (r * npc + (t ^ (w * vx))) * PIECE
                        start(ref.at[ds((g * GH + h0 + h) * SK + off, PIECE, PIECE)],
                              kvbuf.at[slot, h0 + h, w, ds(off, PIECE, PIECE)], sem, w)

        def kv_full(k, v, s):
            slot = lax.rem(s >> 4, NSLOT)
            kv_step(k, v, (s >> 4) & 3, slot, 0, GH, s & 15, kvsem.at[slot])

        def wo_mid(u):
            for t in range(2):
                cs = pl.ds(t * HK, HK)
                for p in range(wo_parts):
                    r = u * 8 + p * (MR // wo_parts)
                    start(ao.at[ds(ER + r, 8, 8), cs], wobuf.at[ds(ER + r, 8, 8), cs], wosem, 0)
                    start(bo.at[ds(r, 8, 8), cs], wobuf.at[ds(D + r, 8, 8), cs], wosem, 1)

        def wo_edge(n):
            pair, kh = n >> 3, (n >> 2) & 1
            cs = ds(kh * HK, HK, HK)
            ra = (1 - pair) * 128
            rb = MR + pair * 128
            sem = (n >> 2) * 2

            def a(r, queue):
                start(ao.at[ds(ra + r, 8, 8), cs], wobuf.at[ds(ra + r, 8, 8), cs], esem.at[sem], queue)

            def b(r, queue):
                start(bo.at[ds(rb + r, 8, 8), cs], wobuf.at[ds(D + rb + r, 8, 8), cs], esem.at[sem + 1], queue)

            def paired():
                for t in range(2):
                    for hh in range(2):
                        a((n & 3) * 16 + t * 8 + hh * 64, 0)
                        b((n & 3) * 16 + t * 8 + hh * 64, 1)

            def single(f):
                for t in range(4):
                    for hh in range(2):
                        f((n & 1) * 32 + t * 8 + hh * 64, hh)

            if lastsplit:
                pl.when(n < NES - 4)(paired)
                pl.when((n >= NES - 4) & (n < NES - 2))(lambda: single(a))
                pl.when(n >= NES - 2)(lambda: single(b))
            else:
                paired()

        NFULL = NSTEP - 16 if small else NSTEP
        LAST = (NSTEP // 16 - 1) % NSLOT

        def issue(s):
            pl.when(s < NSTEP // 2)(lambda: kv_full(ak, av, s))
            pl.when((s >= NSTEP // 2) & (s < NFULL))(lambda: kv_full(bk, bv, s))
            if small:
                @pl.when((s >= NFULL) & (s < NSTEP))
                def _():
                    sg = (s >> 3) & 1
                    kv_step(bk, bv, 3, LAST, sg * 4, 4, s & 7, kvsem.at[NSLOT + sg])

            @pl.when(s >= NSTEP)
            def _():
                x = s - NSTEP
                lo = jnp.minimum(x + jnp.minimum(x, boost), NU)
                hi = jnp.minimum(x + 1 + jnp.minimum(x + 1, boost), NU)
                lax.fori_loop(lo, hi, lambda u, _: wo_mid(u), None)

        def xstart():
            start(ax, xbuf.at[0], xsem, 0)
            start(bx, xbuf.at[1], xsem, 1)

        if xpos == 0:
            xstart()

        @pl.loop(0, D // wq_parts // 8)
        def _(u):
            for t in range(2):
                cs = pl.ds(t * HK, HK)
                for p in range(wq_parts):
                    rs = ds(u * 8 + p * (D // wq_parts), 8, 8)
                    for i, src in enumerate((aq, bq)):
                        start(src.at[rs, cs], wqbuf.at[i, rs, cs], wqsem, i)

        if xpos == 1:
            xstart()
        xrow = lax.broadcasted_iota(jnp.int32, (8, D), 0)
        QW = 2 * E // 16

        @pl.loop(0, lead + 16)
        def _(s):
            kv_full(ak, av, s)

            @pl.when(s == lead)
            def _():
                wait(xbuf, xsem)
                wait(wqbuf, wqsem)

            if skip & 1:
                return

            @pl.when(s >= lead)
            def _():
                c = s - lead
                x = xbuf[c >> 3].astype(f32)
                x8 = jnp.where((xrow & 1) == 0, x[0:1], x[1:2]).astype(bf16)
                q = jnp.dot(x8, wqbuf[c >> 3, :, ds((c & 7) * QW, QW, QW)], preferred_element_type=f32)
                for t in range(QW // (2 * DH)):
                    q0, q1 = (q[:, n * DH:(n + 1) * DH] for n in (2 * t, 2 * t + 1))
                    qbuf[c * (QW // (2 * DH)) + t] = jnp.where((row & 2) == 0, q0, q1)

        @pl.loop(0, 2 * NH)
        def _(i):
            slot = lax.rem(i >> 3, NSLOT)
            h = i & 7
            s = 2 * i + 16 + lead
            if small:
                s = s - jnp.clip(i - (2 * NH - 16), 0, 8)
                pl.when((h == 0) & (i < 2 * NH - 8))(lambda: wait(kvbuf.at[slot], kvsem.at[slot]))
                for sg in range(2):
                    pl.when(i == 2 * NH - 8 + 4 * sg)(
                        lambda sg=sg: wait(kvbuf.at[LAST, pl.ds(4 * sg, 4)], kvsem.at[NSLOT + sg]))
            else:
                pl.when(h == 0)(lambda: wait(kvbuf.at[slot], kvsem.at[slot]))

            issue(s)
            if not skip & 2:
                q = qbuf[((i >> 5) << 4) + (i & 15)].astype(bf16)
                sc = lax.dot_general(q, kvbuf[slot, h, 0], _NT, preferred_element_type=f32)
                sbuf[...] = sc
                m = jnp.max(sc, axis=1, keepdims=True)
            if small:
                pl.when((i >> 3) != 2 * NH // 8 - 2)(lambda: issue(s + 1))
            else:
                issue(s + 1)
            if not skip & 2:
                p = jnp.exp2((sbuf[...] - m) * C2)
                acc = jnp.dot(p.astype(bf16), kvbuf[slot, h, 1], preferred_element_type=f32)
                obuf[i] = acc / jnp.sum(p, axis=1, keepdims=True)

        dst = outbuf if outdma else o_ref
        lax.fori_loop(0, pre, lambda n, _: wo_edge(n), None)
        for h in range(HKV):
            oa = jnp.where((row & 1) == 0, obuf[h], obuf[HKV + h])
            ob = jnp.where((row & 1) == 0, obuf[NH + h], obuf[NH + HKV + h])
            o = jnp.where(row < 4, oa, ob)
            oall[:, 2 * h * DH:(2 * h + 1) * DH] = jnp.where((row & 2) == 0, o, 0.0).astype(bf16)
            oall[:, (2 * h + 1) * DH:(2 * h + 2) * DH] = jnp.where((row & 2) == 0, 0.0, o).astype(bf16)
        accbuf[...] = jnp.zeros(accbuf.shape, f32)
        lane = lax.broadcasted_iota(jnp.int32, (2, DH), 1)
        wait(wobuf.at[pl.ds(ER, 2 * MR)], wosem)
        NMID = 2 * (NT - 4)

        @pl.loop(0, 2 * NT)
        def _(s):
            if eper == 1:
                pl.when(pre + s < NES)(lambda: wo_edge(pre + s))
            else:
                lax.fori_loop(jnp.minimum(pre + s * eper, NES), jnp.minimum(pre + (s + 1) * eper, NES), lambda n, _: wo_edge(n), None)
            e = s - NMID
            t = jnp.where(e < 0, 2 + (s >> 1), jnp.where((e & 1) == 0, 1 - (e >> 2), NT - 2 + (e >> 2)))
            rows = ds(t * 128, 128, 128)
            cs = ds(jnp.where(e < 0, s & 1, (e >> 1) & 1) * HK, HK, HK)
            pl.when(e >= 0)(lambda: wait(wobuf.at[rows, cs], esem.at[e]))
            if skip & 4:
                dst[:, rows] = jnp.zeros((2, 128), bf16)
                return
            r = accbuf[t] + lax.dot_general(oall[:, cs], wobuf[rows, cs], _NT, preferred_element_type=f32)
            accbuf[t] = r
            dst[:, rows] = jnp.where(lane + t * 128 < D, r[0:2] + r[2:4], r[4:6] + r[6:8]).astype(bf16)

        if outdma:
            cp = pltpu.make_async_copy(outbuf, o_ref, osem)
            cp.start()
            cp.wait()

    @jax.jit
    def fn(A_x, A_k_cache, A_v_cache, A_wq, A_wo, B_x, B_k_cache, B_v_cache, B_wq, B_wo):
        rows = lambda t: t.reshape(-1, DH)
        hbm = pl.BlockSpec(memory_space=pltpu.HBM)
        dma = pltpu.SemaphoreType.DMA
        out = pl.pallas_call(
            kernel,
            out_shape=jax.ShapeDtypeStruct((B, 2 * D), bf16),
            in_specs=[hbm] * 10,
            out_specs=hbm if outdma else pl.BlockSpec(memory_space=pltpu.VMEM),
            scratch_shapes=[
                pltpu.VMEM((2, B, D), bf16),
                pltpu.VMEM((2, D, E), bf16),
                pltpu.VMEM((2 * D, E), bf16),
                pltpu.VMEM((NSLOT, GH, 2, SK, DH), bf16),
                pltpu.VMEM((2 * HKV, 8, DH), f32),
                pltpu.VMEM((8, SK), f32),
                pltpu.VMEM((2 * NH, 8, DH), f32),
                pltpu.VMEM((8, E), bf16),
                pltpu.VMEM((NT, 8, DH), f32),
                pltpu.VMEM((B, 2 * D), bf16),
                dma(()), dma(()), dma(()), dma((NSLOT + 2,)), dma((8,)), dma(()),
            ],
            compiler_params=pltpu.CompilerParams(vmem_limit_bytes=100 * 2**20, disable_bounds_checks=nobc),
        )(A_x.reshape(B, D), rows(A_k_cache), rows(A_v_cache), A_wq, A_wo.T,
          B_x.reshape(B, D), rows(B_k_cache), rows(B_v_cache), B_wq, B_wo.T)
        return out.reshape(B, 1, 2 * D)

    return fn


_fn = make(**{})


@jax.jit
def pallas_concat_heads__gqa_block_cached__gqa_block_cached__decode_kernel(
        A_x, A_k_cache, A_v_cache, A_wq, A_wo, B_x, B_k_cache, B_v_cache, B_wq, B_wo):
    return _fn(A_x, A_k_cache, A_v_cache, A_wq, A_wo, B_x, B_k_cache, B_v_cache, B_wq, B_wo)
```

```python
import math

import jax
import jax.numpy as jnp
from jax import lax
import jax.experimental.pallas as pl
import jax.experimental.pallas.tpu as pltpu

_NT = (((1,), (1,)), ((), ()))


def make(vx=1, wq_parts=4, wo_parts=4, pre=4, lead=2, boost=2, skip=0, xpos=1, outdma=False,
         nobc=True, sh='00000000'):
    B, D, HQ, HKV, SK, DH = 2, 576, 32, 16, 4096, 128
    E = HQ * DH
    NH = B * HKV
    GH, NSLOT, PIECE = 8, 3, 128
    NSTEP = 4 * NH
    C2 = (DH ** -0.5) * math.log2(math.e)
    NT = 2 * D // 128
    ER = 256
    MR = D - ER
    NU = MR // 8 // wo_parts
    HK = E // 2
    NES = 16
    sak, sav, saq, sao, sbk, sbv, sbq, sbo = (int(c) for c in sh)
    QK = E // 4
    f32, bf16 = jnp.float32, jnp.bfloat16

    def ds(start, size, align):
        return pl.ds(pl.multiple_of(start, align), size)

    def kernel(ax, ak, av, aq, ao, bx, bk, bv, bq, bo, o_ref,
               xbuf, wqbuf, wobuf, kvbuf, qbuf, sbuf, obuf, oall, accbuf, outbuf, xsem, wqsem, wosem, kvsem, esem, osem):
        row = lax.broadcasted_iota(jnp.int32, (8, DH), 0)

        def start(src, dst, sem, queue):
            pltpu.make_async_copy(src, dst, sem).start(priority=queue)

        def wait(buf, sem):
            pltpu.make_async_copy(buf, buf, sem).wait()

        def kv_step(k, v, g, slot, h0, nh, r, sem):
            npc = 16 // nh
            for t in range(npc):
                for h in range(nh):
                    for w, (ref, phase) in enumerate((k, v)):
                        tt = t ^ (w * vx)
                        off = h * SK + (r * npc + tt) * PIECE + phase * (PIECE // 2)
                        parts = [(off, PIECE)]
                        if phase and h == nh - 1 and tt == npc - 1:
                            parts = [(off, PIECE // 2), ((off + PIECE // 2) & (nh * SK - 1), PIECE // 2)]
                        for o, n in parts:
                            start(ref.at[ds((g * GH + h0) * SK + o, n, PIECE // 2)],
                                  kvbuf.at[slot, w, ds(h0 * SK + o, n, PIECE // 2)], sem, w)

        def w_piece(src, phase, dst, d0, r0, u, nu, t, sem, queue):
            def go(uu, c, cd, n):
                start(src.at[ds(r0 + uu * 8, 8, 8), pl.ds(c, n)], dst.at[ds(d0 + r0 + uu * 8, 8, 8), pl.ds(cd, n)], sem, queue)
            if not phase:
                go(u, t * HK, t * HK, HK)
            elif t == 0:
                go(u, QK, 0, HK)
            else:
                go(u, 3 * QK, 2 * QK, QK)
                go(jnp.where(u + 1 == nu, 0, u + 1), 0, 3 * QK, QK)

        akv, bkv = ((ak, sak), (av, sav)), ((bk, sbk), (bv, sbv))

        def kv_full(k, v, s):
            slot = lax.rem(s >> 4, NSLOT)
            kv_step(k, v, (s >> 4) & 3, slot, 0, GH, s & 15, kvsem.at[slot])

        def wo_mid(u):
            for t in range(2):
                for p in range(wo_parts):
                    r = p * (MR // wo_parts)
                    w_piece(ao, sao, wobuf, 0, ER + r, u, NU, t, wosem, 0)
                    w_piece(bo, sbo, wobuf, D, r, u, NU, t, wosem, 1)

        def wo_edge(n):
            pair = n >> 3
            sem = (n >> 2) * 2
            def go(kh):
                for t in range(2):
                    for hh in range(2):
                        u = (n & 3) * 2 + t
                        w_piece(ao, sao, wobuf, 0, (1 - pair) * 128 + hh * 64, u, 8, kh, esem.at[sem], 0)
                        w_piece(bo, sbo, wobuf, D, MR + pair * 128 + hh * 64, u, 8, kh, esem.at[sem + 1], 1)
            pl.when((n & 4) == 0)(lambda: go(0))
            pl.when((n & 4) != 0)(lambda: go(1))

        NFULL = NSTEP - 16
        LAST = (NSTEP // 16 - 1) % NSLOT

        def issue(s):
            pl.when(s < NSTEP // 2)(lambda: kv_full(*akv, s))
            pl.when((s >= NSTEP // 2) & (s < NFULL))(lambda: kv_full(*bkv, s))
            if True:
                @pl.when((s >= NFULL) & (s < NSTEP))
                def _():
                    sg = (s >> 3) & 1
                    kv_step(*bkv, 3, LAST, sg * 4, 4, s & 7, kvsem.at[NSLOT + sg])

            @pl.when(s >= NSTEP)
            def _():
                x = s - NSTEP
                lo = jnp.minimum(x + jnp.minimum(x, boost), NU)
                hi = jnp.minimum(x + 1 + jnp.minimum(x + 1, boost), NU)
                lax.fori_loop(lo, hi, lambda u, _: wo_mid(u), None)

        def xstart():
            start(ax, xbuf.at[0], xsem, 0)
            start(bx, xbuf.at[1], xsem, 1)

        if xpos == 0:
            xstart()

        @pl.loop(0, D // wq_parts // 8)
        def _(u):
            for t in range(2):
                for p in range(wq_parts):
                    for i, (src, phase) in enumerate(((aq, saq), (bq, sbq))):
                        w_piece(src, phase, wqbuf.at[i], 0, p * (D // wq_parts), u, D // wq_parts // 8, t, wqsem, i)

        if xpos == 1:
            xstart()
        xrow = lax.broadcasted_iota(jnp.int32, (8, D), 0)
        QW = 2 * E // 16

        @pl.loop(0, lead + 16)
        def _(s):
            kv_full(*akv, s)

            @pl.when(s == lead)
            def _():
                wait(xbuf, xsem)
                wait(wqbuf, wqsem)

            if skip & 1:
                return

            @pl.when(s >= lead)
            def _():
                c = s - lead
                x = xbuf[c >> 3].astype(f32)
                x8 = jnp.where((xrow & 1) == 0, x[0:1], x[1:2]).astype(bf16)
                q = jnp.dot(x8, wqbuf[c >> 3, :, ds((c & 7) * QW, QW, QW)], preferred_element_type=f32)
                for t in range(QW // (2 * DH)):
                    q0, q1 = (q[:, n * DH:(n + 1) * DH] for n in (2 * t, 2 * t + 1))
                    qbuf[c * (QW // (2 * DH)) + t] = jnp.where((row & 2) == 0, q0, q1)

        @pl.loop(0, 2 * NH)
        def _(i):
            slot = lax.rem(i >> 3, NSLOT)
            h = i & 7
            s = 2 * i + 16 + lead
            if True:
                s = s - jnp.clip(i - (2 * NH - 16), 0, 8)
                pl.when((h == 0) & (i < 2 * NH - 8))(lambda: wait(kvbuf.at[slot], kvsem.at[slot]))
                for sg in range(2):
                    pl.when(i == 2 * NH - 8 + 4 * sg)(
                        lambda sg=sg: wait(kvbuf.at[LAST, :, pl.ds(4 * sg * SK, 4 * SK)], kvsem.at[NSLOT + sg]))

            issue(s)
            if not skip & 2:
                q = qbuf[((i >> 5) << 4) + ((i - 4 * jnp.where(i < NH, saq, sbq)) & 15)].astype(bf16)
                sc = lax.dot_general(q, kvbuf[slot, 0, ds(h * SK, SK, SK)], _NT, preferred_element_type=f32)
                sbuf[...] = sc
                m = jnp.max(sc, axis=1, keepdims=True)
            if True:
                pl.when((i >> 3) != 2 * NH // 8 - 2)(lambda: issue(s + 1))
            if not skip & 2:
                p = jnp.exp2((sbuf[...] - m) * C2)
                acc = jnp.dot(p.astype(bf16), kvbuf[slot, 1, ds(h * SK, SK, SK)], preferred_element_type=f32)
                obuf[i] = acc / jnp.sum(p, axis=1, keepdims=True)

        dst = outbuf if outdma else o_ref
        lax.fori_loop(0, pre, lambda n, _: wo_edge(n), None)
        for h in range(HKV):
            oa = jnp.where((row & 1) == 0, obuf[(h + 4 * sao) % HKV], obuf[HKV + (h + 4 * sao) % HKV])
            ob = jnp.where((row & 1) == 0, obuf[NH + (h + 4 * sbo) % HKV], obuf[NH + HKV + (h + 4 * sbo) % HKV])
            o = jnp.where(row < 4, oa, ob)
            oall[:, 2 * h * DH:(2 * h + 1) * DH] = jnp.where((row & 2) == 0, o, 0.0).astype(bf16)
            oall[:, (2 * h + 1) * DH:(2 * h + 2) * DH] = jnp.where((row & 2) == 0, 0.0, o).astype(bf16)
        accbuf[...] = jnp.zeros(accbuf.shape, f32)
        lane = lax.broadcasted_iota(jnp.int32, (2, DH), 1)
        wait(wobuf.at[pl.ds(ER, 2 * MR)], wosem)
        NMID = 2 * (NT - 4)

        @pl.loop(0, 2 * NT)
        def _(s):
            pl.when(pre + s < NES)(lambda: wo_edge(pre + s))
            e = s - NMID
            t = jnp.where(e < 0, 2 + (s >> 1), jnp.where((e & 1) == 0, 1 - (e >> 2), NT - 2 + (e >> 2)))
            rows = ds(t * 128, 128, 128)
            cs = ds(jnp.where(e < 0, s & 1, (e >> 1) & 1) * HK, HK, HK)
            pl.when(e >= 0)(lambda: wait(wobuf.at[rows, cs], esem.at[e]))
            if skip & 4:
                dst[:, rows] = jnp.zeros((2, 128), bf16)
                return
            r = accbuf[t] + lax.dot_general(oall[:, cs], wobuf[rows, cs], _NT, preferred_element_type=f32)
            accbuf[t] = r
            dst[:, rows] = jnp.where(lane + t * 128 < D, r[0:2] + r[2:4], r[4:6] + r[6:8]).astype(bf16)

        if outdma:
            cp = pltpu.make_async_copy(outbuf, o_ref, osem)
            cp.start()
            cp.wait()

    @jax.jit
    def fn(A_x, A_k_cache, A_v_cache, A_wq, A_wo, B_x, B_k_cache, B_v_cache, B_wq, B_wo):
        rows = lambda t: t.reshape(-1, DH)
        hbm = pl.BlockSpec(memory_space=pltpu.HBM)
        dma = pltpu.SemaphoreType.DMA
        out = pl.pallas_call(
            kernel,
            out_shape=jax.ShapeDtypeStruct((B, 2 * D), bf16),
            in_specs=[hbm] * 10,
            out_specs=hbm if outdma else pl.BlockSpec(memory_space=pltpu.VMEM),
            scratch_shapes=[
                pltpu.VMEM((2, B, D), bf16),
                pltpu.VMEM((2, D, E), bf16),
                pltpu.VMEM((2 * D, E), bf16),
                pltpu.VMEM((NSLOT, 2, GH * SK, DH), bf16),
                pltpu.VMEM((2 * HKV, 8, DH), f32),
                pltpu.VMEM((8, SK), f32),
                pltpu.VMEM((2 * NH, 8, DH), f32),
                pltpu.VMEM((8, E), bf16),
                pltpu.VMEM((NT, 8, DH), f32),
                pltpu.VMEM((B, 2 * D), bf16),
                dma(()), dma(()), dma(()), dma((NSLOT + 2,)), dma((8,)), dma(()),
            ],
            compiler_params=pltpu.CompilerParams(vmem_limit_bytes=100 * 2**20, disable_bounds_checks=nobc),
        )(A_x.reshape(B, D), rows(A_k_cache), rows(A_v_cache), A_wq, A_wo.T,
          B_x.reshape(B, D), rows(B_k_cache), rows(B_v_cache), B_wq, B_wo.T)
        return out.reshape(B, 1, 2 * D)

    return fn


_fn = make(**dict(sh='00001100'))


@jax.jit
def pallas_concat_heads__gqa_block_cached__gqa_block_cached__decode_kernel(
        A_x, A_k_cache, A_v_cache, A_wq, A_wo, B_x, B_k_cache, B_v_cache, B_wq, B_wo):
    return _fn(A_x, A_k_cache, A_v_cache, A_wq, A_wo, B_x, B_k_cache, B_v_cache, B_wq, B_wo)
```

```python
import math

import jax
import jax.numpy as jnp
import numpy as np
from jax import lax
import jax.experimental.pallas as pl
import jax.experimental.pallas.tpu as pltpu

_NT = (((1,), (1,)), ((), ()))


def make(sh='01', hc=32, mix=1, wq_parts=4, wo_parts=4, pre=4, lead=1, nq=4, skip=0, cuts=(0, 2048, 3072, 4096), outdma=False, nobc=True, isub=2):
    B, D, HQ, HKV, SK, DH = 2, 576, 32, 16, 4096, 128
    E = HQ * DH
    NH = B * HKV
    PIECE = 128
    NCH = NH // hc
    NSTEP = 2 * NCH * (SK // PIECE)
    AHEAD = lead + nq
    NSLOT = 1 << AHEAD.bit_length()
    C2 = (DH ** -0.5) * math.log2(math.e)
    NT = 2 * D // 128
    ER = 256
    MR = D - ER
    NU = MR // 8 // wo_parts
    HK, QK = E // 2, E // 4
    KW = min(b - a for a, b in zip(cuts, cuts[1:]))
    NPH = len(cuts) - 1
    assert all(8 % (-(-b // 512) - a // 512) == 0 for a, b in zip(cuts, cuts[1:])) and NU * 8 * wo_parts == MR
    sak, sbk = (int(c) for c in sh)
    f32, bf16 = jnp.float32, jnp.bfloat16
    lg = lambda n: n.bit_length() - 1

    def ds(start, size, align):
        return pl.ds(pl.multiple_of(start, align), size)

    def decode(s):
        chunk = s & (NCH - 1)
        j = s >> lg(NCH)
        if mix:
            return j & 1, chunk, j >> 1
        return j >> 5, chunk, j & 31

    def kernel(ax, ak, av, aq, ao, bx, bk, bv, bq, bo, o_ref,
               xbuf, wqbuf, wobuf, kvbuf, qbuf, mbuf, lbuf, obuf, oall, accbuf, outbuf, xsem, wqsem, wosem, kvsem, esem, osem):
        row = lax.broadcasted_iota(jnp.int32, (8, DH), 0)

        def start(src, dst, sem, queue):
            pltpu.make_async_copy(src, dst, sem).start(priority=queue)

        def wait(buf, sem):
            pltpu.make_async_copy(buf, buf, sem).wait()

        def kv_step(k, v, phase, chunk, r, slot):
            HP = PIECE // 2
            base = chunk * (hc * SK)
            d = jnp.where(r == SK // PIECE - 1, HP, 0) if phase else 0
            for h in range(hc):
                so, do = h * SK + r * PIECE + phase * HP, h * PIECE + d
                parts = [(so, do, PIECE)]
                if phase and h == hc - 1:
                    parts = [(so, do, HP), ((so + HP) & (hc * SK - 1), (do + HP) & (hc * PIECE - 1), HP)]
                for w, ref in enumerate((k, v)):
                    for a, b, n in parts:
                        start(ref.at[ds(base + a, n, HP)], kvbuf.at[slot, w, ds(b, n, HP) if phase else pl.ds(b, n)], kvsem.at[slot], w)

        def kv_issue(s):
            br, chunk, r = decode(s)
            pl.when(br == 0)(lambda: kv_step(ak, av, sak, chunk, r, s & (NSLOT - 1)))
            pl.when(br == 1)(lambda: kv_step(bk, bv, sbk, chunk, r, s & (NSLOT - 1)))

        def w_piece(src, dst, d0, r, cs, sem, queue):
            start(src.at[ds(r, 8, 8), cs], dst.at[ds(d0 + r, 8, 8), cs], sem, queue)

        def wo_mid(u):
            for t in range(2):
                for p in range(wo_parts):
                    r = p * (MR // wo_parts) + u * 8
                    w_piece(ao, wobuf, 0, ER + r, pl.ds(t * HK, HK), wosem, 0)
                    w_piece(bo, wobuf, D, r, pl.ds(t * HK, HK), wosem, 1)

        def wo_edge(pair, u, nu, cs, sem):
            for t in range(nu):
                for hh in range(2):
                    r = hh * 64 + (u * nu + t) * 8
                    w_piece(ao, wobuf, 0, (1 - pair) * 128 + r, cs, sem, 0)
                    w_piece(bo, wobuf, D, MR + pair * 128 + r, cs, sem, 1)

        def edge_slot(n):
            pl.when(n < 8)(lambda: wo_edge(0, n & 3, 2, ds((n >> 2) * HK, HK, HK), esem.at[NPH]))
            for ph, (c0, c1) in enumerate(zip(cuts, cuts[1:])):
                n0, n1 = 8 + c0 // 512, 8 + -(-c1 // 512)
                pl.when((n >= n0) & (n < n1))(
                    lambda ph=ph, c0=c0, c1=c1, n0=n0, n1=n1: wo_edge(1, n - n0, 8 // (n1 - n0), pl.ds(c0, c1 - c0), esem.at[ph]))

        @pl.loop(0, D // wq_parts // 8)
        def _(u):
            for t in range(2):
                for p in range(wq_parts):
                    for i, src in enumerate((aq, bq)):
                        w_piece(src, wqbuf.at[i], 0, p * (D // wq_parts) + u * 8, pl.ds(t * HK, HK), wqsem, i)

        start(ax, xbuf.at[0], xsem, 0)
        start(bx, xbuf.at[1], xsem, 1)
        mbuf[...] = jnp.full(mbuf.shape, float(np.finfo(np.float32).min), f32)
        lbuf[...] = jnp.zeros(lbuf.shape, f32)
        obuf[...] = jnp.zeros(obuf.shape, f32)
        xrow = lax.broadcasted_iota(jnp.int32, (8, D), 0)
        QW = 2 * E // nq

        @pl.loop(0, NSTEP + AHEAD)
        def _(n):
            pl.when(n < NSTEP)(lambda: kv_issue(n))

            @pl.when(n >= NSTEP)
            def _():
                x = n - NSTEP
                per = -(-NU // AHEAD)
                lax.fori_loop(jnp.minimum(x * per, NU), jnp.minimum((x + 1) * per, NU), lambda u, _: wo_mid(u), None)

            @pl.when(n == lead)
            def _():
                wait(xbuf, xsem)
                wait(wqbuf, wqsem)

            @pl.when((n >= lead) & (n < AHEAD))
            def _():
                if skip & 1:
                    return
                c = n - lead
                br, cc = c >> lg(nq // 2), c & (nq // 2 - 1)
                x = xbuf[br].astype(f32)
                x8 = jnp.where((xrow & 1) == 0, x[0:1], x[1:2]).astype(bf16)
                q = jnp.dot(x8, wqbuf[br, :, ds(cc * QW, QW, QW)], preferred_element_type=f32)
                for t in range(QW // (2 * DH)):
                    q0, q1 = (q[:, i * DH:(i + 1) * DH] for i in (2 * t, 2 * t + 1))
                    qbuf[c * (QW // (2 * DH)) + t] = jnp.where((row & 2) == 0, q0, q1)

            @pl.when(n >= AHEAD)
            def _():
                s = n - AHEAD
                slot = s & (NSLOT - 1)
                wait(kvbuf.at[slot], kvsem.at[slot])
                if skip & 2:
                    return
                br, chunk, _ = decode(s)
                st = pl.ds(br * NH + chunk * hc, hc)
                q0 = br * HKV + ((chunk * hc) & (HKV - 1))
                sc = jnp.stack([
                    lax.dot_general(qbuf[q0 + h % HKV].astype(bf16), kvbuf[slot, 0, h * PIECE:(h + 1) * PIECE], _NT,
                                    preferred_element_type=f32) for h in range(hc)])
                m_old = mbuf[st]
                m = jnp.maximum(m_old, jnp.max(sc, axis=2, keepdims=True))
                alpha = jnp.exp2((m_old - m) * C2)
                p = jnp.exp2((sc - m) * C2)
                mbuf[st] = m
                lbuf[st] = lbuf[st] * alpha + p
                pv = jnp.stack([
                    jnp.dot(p[h].astype(bf16), kvbuf[slot, 1, h * PIECE:(h + 1) * PIECE], preferred_element_type=f32)
                    for h in range(hc)])
                obuf[st] = obuf[st] * alpha + pv

        dst = outbuf if outdma else o_ref
        lax.fori_loop(0, pre, lambda n, _: edge_slot(n), None)
        on = obuf[...] / jnp.sum(lbuf[...], axis=2, keepdims=True)
        for h in range(HKV):
            ha, hb = h, NH + h
            o = jnp.where(row < 4, jnp.where((row & 1) == 0, on[ha], on[HKV + ha]), jnp.where((row & 1) == 0, on[hb], on[HKV + hb]))
            oall[:, 2 * h * DH:(2 * h + 1) * DH] = jnp.where((row & 2) == 0, o, 0.0).astype(bf16)
            oall[:, (2 * h + 1) * DH:(2 * h + 2) * DH] = jnp.where((row & 2) == 0, 0.0, o).astype(bf16)
        lane = lax.broadcasted_iota(jnp.int32, (2, DH), 1)
        wait(wobuf.at[pl.ds(ER, 2 * MR)], wosem)

        @pl.loop(0, NT - 2)
        def _(s):
            lax.fori_loop(jnp.minimum(pre + s * isub, 16), jnp.minimum(pre + (s + 1) * isub, 16), lambda n, _: edge_slot(n), None)
            t = jnp.where(s < NT - 4, 2 + s, jnp.where(s == NT - 4, 1, NT - 2))
            rows = ds(t * 128, 128, 128)

            @pl.when(s == NT - 4)
            def _():
                for tt in (1, NT - 2):
                    wait(wobuf.at[pl.ds(tt * 128, 128)], esem.at[NPH])

            r = lax.dot_general(oall[...], wobuf[rows, :], _NT, preferred_element_type=f32)
            dst[:, rows] = jnp.where(lane + t * 128 < D, r[0:2] + r[2:4], r[4:6] + r[6:8]).astype(bf16)

        lax.fori_loop(min(pre + (NT - 2) * isub, 16), 16, lambda n, _: edge_slot(n), None)

        @pl.loop(0, NPH)
        def _(j):
            for ph, (c0, c1) in enumerate(zip(cuts, cuts[1:])):
                @pl.when(j == ph)
                def _():
                    for tt in (0, NT - 1):
                        wait(wobuf.at[pl.ds(tt * 128, 128), pl.ds(c0, c1 - c0)], esem.at[ph])
                    r = [lax.dot_general(oall[:, c0:c1], wobuf[tt * 128:(tt + 1) * 128, c0:c1], _NT, preferred_element_type=f32)
                         for tt in (0, NT - 1)]
                    if ph:
                        r = [accbuf[i] + r[i] for i in range(2)]
                    if ph < NPH - 1:
                        accbuf[0], accbuf[1] = r
                    else:
                        dst[:, :128] = (r[0][0:2] + r[0][2:4]).astype(bf16)
                        dst[:, 2 * D - 128:] = (r[1][4:6] + r[1][6:8]).astype(bf16)

        if outdma:
            cp = pltpu.make_async_copy(outbuf, o_ref, osem)
            cp.start()
            cp.wait()

    @jax.jit
    def fn(A_x, A_k_cache, A_v_cache, A_wq, A_wo, B_x, B_k_cache, B_v_cache, B_wq, B_wo):
        rows = lambda t: t.reshape(-1, DH)
        hbm = pl.BlockSpec(memory_space=pltpu.HBM)
        dma = pltpu.SemaphoreType.DMA
        state = pltpu.VMEM((2 * NH, 8, DH), f32)
        out = pl.pallas_call(
            kernel,
            out_shape=jax.ShapeDtypeStruct((B, 2 * D), bf16),
            in_specs=[hbm] * 10,
            out_specs=hbm if outdma else pl.BlockSpec(memory_space=pltpu.VMEM),
            scratch_shapes=[
                pltpu.VMEM((2, B, D), bf16),
                pltpu.VMEM((2, D, E), bf16),
                pltpu.VMEM((2 * D, E), bf16),
                pltpu.VMEM((NSLOT, 2, hc * PIECE, DH), bf16),
                pltpu.VMEM((2 * HKV, 8, DH), f32),
                state, state, state,
                pltpu.VMEM((8, E), bf16),
                pltpu.VMEM((2, 8, DH), f32),
                pltpu.VMEM((B, 2 * D), bf16),
                dma(()), dma(()), dma(()), dma((NSLOT,)), dma((1 + NPH,)), dma(()),
            ],
            compiler_params=pltpu.CompilerParams(vmem_limit_bytes=64 * 2**20, disable_bounds_checks=nobc),
        )(A_x.reshape(B, D), rows(A_k_cache), rows(A_v_cache), A_wq, A_wo.T,
          B_x.reshape(B, D), rows(B_k_cache), rows(B_v_cache), B_wq, B_wo.T)
        return out.reshape(B, 1, 2 * D)

    return fn


_fn = make(**{})


@jax.jit
def pallas_concat_heads__gqa_block_cached__gqa_block_cached__decode_kernel(
        A_x, A_k_cache, A_v_cache, A_wq, A_wo, B_x, B_k_cache, B_v_cache, B_wq, B_wo):
    return _fn(A_x, A_k_cache, A_v_cache, A_wq, A_wo, B_x, B_k_cache, B_v_cache, B_wq, B_wo)
```

```python
import math

import jax
import jax.numpy as jnp
import numpy as np
from jax import lax
import jax.experimental.pallas as pl
import jax.experimental.pallas.tpu as pltpu

B, D, HQ, HKV, SK, DH = 2, 576, 32, 16, 4096, 128
E = HQ * DH
NH = B * HKV
BLK = 128
NSTEP = 2 * (SK // BLK)
NQ = 4
AHEAD = 1 + NQ
NSLOT = 8
PARTS = 4
MID = D - 256
NMID = MID // 8 // PARTS
NTILE = 2 * D // 128
TAIL = (0, 2048, 3072, 4096)
PHASE = (0, 1)
EXP2_SCALE = DH ** -0.5 * math.log2(math.e)
NEG = float(np.finfo(np.float32).min)
NT_DIMS = (((1,), (1,)), ((), ()))


def _ds(start, size, align):
    return pl.ds(start if isinstance(start, int) else pl.multiple_of(start, align), size)


def _start(src, dst, sem, queue):
    pltpu.make_async_copy(src, dst, sem).start(priority=queue)


def _wait_filled(buf, sem):
    pltpu.make_async_copy(buf, buf, sem).wait()


def _fetch_rows(src, dst, src_row, dst_row, u, nu, half, phase, sem, queue):
    def copy(g, col, width):
        cols = pl.ds(col, width)
        _start(src.at[_ds(src_row + g * 8, 8, 8), cols], dst.at[_ds(dst_row + g * 8, 8, 8), cols], sem, queue)

    if not phase:
        copy(u, half * (E // 2), E // 2)
    elif half == 0:
        copy(u, E // 4, E // 2)
    else:
        copy(u, 3 * E // 4, E // 4)
        copy(jnp.where(u + 1 == nu, 0, u + 1), 0, E // 4)


def _fetch_kv(k, v, phase, blk, dst, sem):
    half = BLK // 2
    wrap = jnp.where(blk == SK // BLK - 1, half, 0) if phase else 0
    for h in range(NH):
        src_row, dst_row = h * SK + blk * BLK + phase * half, h * BLK + wrap
        parts = [(src_row, dst_row, BLK)]
        if phase and h == NH - 1:
            parts = [(src_row, dst_row, half),
                     ((src_row + half) & (NH * SK - 1), (dst_row + half) & (NH * BLK - 1), half)]
        for i, ref in enumerate((k, v)):
            for a, b, n in parts:
                _start(ref.at[_ds(a, n, half)], dst.at[i, _ds(b, n, half)], sem, i)


def _kernel(ax, ak, av, aq, ao, bx, bk, bv, bq, bo, out_ref,
            xbuf, wqbuf, kvbuf, wobuf, tail0, tail1, tail2, qbuf, mbuf, lbuf, obuf, oall, tacc,
            xsem, wqsem, kvsem, wosem, tsem):
    f32, bf16 = jnp.float32, jnp.bfloat16
    tails = (tail0, tail1, tail2)
    row = lax.broadcasted_iota(jnp.int32, (8, DH), 0)

    def fetch_wo_mid(u):
        for half in range(2):
            for p in range(PARTS):
                r = p * (MID // PARTS)
                _fetch_rows(ao, wobuf, D - MID + r, r, u, NMID, half, PHASE[0], wosem.at[0], 0)
                _fetch_rows(bo, wobuf, r, MID + r, u, NMID, half, PHASE[1], wosem.at[0], 1)

    def fetch_wo_edge(n):
        @pl.when(n < 8)
        def _():
            for half in range(2):
                for r in (0, 64):
                    _fetch_rows(ao, wobuf, 128 + r, 2 * MID + r, n, 8, half, 0, wosem.at[1], 0)
                    _fetch_rows(bo, wobuf, MID + r, 2 * MID + 128 + r, n, 8, half, 0, wosem.at[1], 1)

        for i, buf in enumerate(tails):
            first, last = 8 + TAIL[i] // 512, 8 + TAIL[i + 1] // 512
            per = 8 // (last - first)
            cols = pl.ds(TAIL[i], TAIL[i + 1] - TAIL[i])

            @pl.when((n >= first) & (n < last))
            def _():
                for t in range(per):
                    for r0 in (0, 64):
                        r = r0 + ((n - first) * per + t) * 8
                        _start(ao.at[_ds(r, 8, 8), cols], buf.at[_ds(r, 8, 8)], tsem.at[i], 0)
                        _start(bo.at[_ds(D - 128 + r, 8, 8), cols], buf.at[_ds(128 + r, 8, 8)], tsem.at[i], 1)

    def project_q(c):
        width = 2 * E // NQ
        branch = c >> 1
        x = xbuf[branch].astype(f32)
        xrow = lax.broadcasted_iota(jnp.int32, (8, D), 0)
        x8 = jnp.where((xrow & 1) == 0, x[0:1], x[1:2]).astype(bf16)
        q = jnp.dot(x8, wqbuf[branch, :, _ds((c & 1) * width, width, width)], preferred_element_type=f32)
        for g in range(width // (2 * DH)):
            q0, q1 = (q[:, i * DH:(i + 1) * DH] for i in (2 * g, 2 * g + 1))
            qbuf[c * (width // (2 * DH)) + g] = jnp.where((row & 2) == 0, q0, q1)

    def attend(branch, slot):
        state = pl.ds(branch * NH, NH)
        s = jnp.stack([
            lax.dot_general(qbuf[branch * HKV + h % HKV].astype(bf16), kvbuf[slot, 0, h * BLK:(h + 1) * BLK],
                            NT_DIMS, preferred_element_type=f32)
            for h in range(NH)])
        m_old = mbuf[state]
        m = jnp.maximum(m_old, jnp.max(s, axis=2, keepdims=True))
        alpha = jnp.exp2((m_old - m) * EXP2_SCALE)
        p = jnp.exp2((s - m) * EXP2_SCALE)
        mbuf[state] = m
        lbuf[state] = lbuf[state] * alpha + p
        pv = jnp.stack([
            jnp.dot(p[h].astype(bf16), kvbuf[slot, 1, h * BLK:(h + 1) * BLK], preferred_element_type=f32)
            for h in range(NH)])
        obuf[state] = obuf[state] * alpha + pv

    @pl.loop(0, D // PARTS // 8)
    def _(u):
        for half in range(2):
            for p in range(PARTS):
                for i, src in enumerate((aq, bq)):
                    r = p * (D // PARTS)
                    _fetch_rows(src, wqbuf.at[i], r, r, u, D // PARTS // 8, half, PHASE[i], wqsem, i)

    xcopies = [pltpu.make_async_copy(src, xbuf.at[i], xsem.at[i]) for i, src in enumerate((ax, bx))]
    for copy in xcopies:
        copy.start()
    mbuf[...] = jnp.full(mbuf.shape, NEG, f32)
    lbuf[...] = jnp.zeros(lbuf.shape, f32)
    obuf[...] = jnp.zeros(obuf.shape, f32)

    @pl.loop(0, NSTEP + AHEAD)
    def _(n):
        for i, (k, v) in enumerate(((ak, av), (bk, bv))):
            @pl.when((n < NSTEP) & ((n & 1) == i))
            def _():
                slot = n & (NSLOT - 1)
                _fetch_kv(k, v, PHASE[i], n >> 1, kvbuf.at[slot], kvsem.at[slot])

        @pl.when(n >= NSTEP)
        def _():
            @pl.loop(0, NMID // AHEAD)
            def _(t):
                fetch_wo_mid((n - NSTEP) * (NMID // AHEAD) + t)

        @pl.when(n == AHEAD - NQ)
        def _():
            for copy in xcopies:
                copy.wait()
            _wait_filled(wqbuf, wqsem)

        @pl.when((n >= AHEAD - NQ) & (n < AHEAD))
        def _():
            project_q(n - (AHEAD - NQ))

        @pl.when(n >= AHEAD)
        def _():
            step = n - AHEAD
            slot = step & (NSLOT - 1)
            _wait_filled(kvbuf.at[slot], kvsem.at[slot])
            attend(step & 1, slot)

    @pl.loop(0, 4)
    def _(n):
        fetch_wo_edge(n)

    o = obuf[...] / jnp.sum(lbuf[...], axis=2, keepdims=True)
    for g in range(HKV):
        oa, ob = (jnp.where((row & 1) == 0, o[i * NH + g], o[i * NH + HKV + g]) for i in range(2))
        og = jnp.where(row < 4, oa, ob)
        oall[:, 2 * g * DH:(2 * g + 1) * DH] = jnp.where((row & 2) == 0, og, 0.0).astype(bf16)
        oall[:, (2 * g + 1) * DH:(2 * g + 2) * DH] = jnp.where((row & 2) == 0, 0.0, og).astype(bf16)

    lane = lax.broadcasted_iota(jnp.int32, (B, 128), 1)
    _wait_filled(wobuf.at[pl.ds(0, 2 * MID)], wosem.at[0])

    @pl.loop(0, NTILE - 2)
    def _(i):
        @pl.when(i < 6)
        def _():
            @pl.loop(0, 2)
            def _(t):
                fetch_wo_edge(4 + 2 * i + t)

        @pl.when(i == NTILE - 4)
        def _():
            _wait_filled(wobuf.at[pl.ds(2 * MID, 256)], wosem.at[1])

        col = jnp.where(i < NTILE - 4, i + 2, jnp.where(i == NTILE - 4, 1, NTILE - 2)) * 128
        r = lax.dot_general(oall[...], wobuf[_ds(i * 128, 128, 128), :], NT_DIMS, preferred_element_type=f32)
        out_ref[:, _ds(col, 128, 128)] = jnp.where(lane + col < D, r[0:2] + r[2:4], r[4:6] + r[6:8]).astype(bf16)

    @pl.loop(0, len(tails))
    def _(j):
        for i, buf in enumerate(tails):
            @pl.when(j == i)
            def _():
                _wait_filled(buf, tsem.at[i])
                r = lax.dot_general(oall[:, TAIL[i]:TAIL[i + 1]], buf[...], NT_DIMS, preferred_element_type=f32)
                if i > 0:
                    r = r + tacc[...]
                if i < len(tails) - 1:
                    tacc[...] = r
                else:
                    out_ref[:, :128] = (r[0:2, :128] + r[2:4, :128]).astype(bf16)
                    out_ref[:, 2 * D - 128:] = (r[4:6, 128:] + r[6:8, 128:]).astype(bf16)


@jax.jit
def pallas_concat_heads__gqa_block_cached__gqa_block_cached__decode_kernel(
    A_x: jax.Array,
    A_k_cache: jax.Array,
    A_v_cache: jax.Array,
    A_wq: jax.Array,
    A_wo: jax.Array,
    B_x: jax.Array,
    B_k_cache: jax.Array,
    B_v_cache: jax.Array,
    B_wq: jax.Array,
    B_wo: jax.Array,
):
    f32, bf16 = jnp.float32, jnp.bfloat16
    dma = pltpu.SemaphoreType.DMA
    state = pltpu.VMEM((2 * NH, 8, DH), f32)
    out = pl.pallas_call(
        _kernel,
        out_shape=jax.ShapeDtypeStruct((B, 2 * D), bf16),
        in_specs=[pl.BlockSpec(memory_space=pltpu.HBM)] * 10,
        out_specs=pl.BlockSpec(memory_space=pltpu.VMEM),
        scratch_shapes=[
            pltpu.VMEM((2, B, D), bf16),
            pltpu.VMEM((2, D, E), bf16),
            pltpu.VMEM((NSLOT, 2, NH * BLK, DH), bf16),
            pltpu.VMEM(((NTILE - 2) * 128, E), bf16),
            *[pltpu.VMEM((256, b - a), bf16) for a, b in zip(TAIL, TAIL[1:])],
            pltpu.VMEM((2 * HKV, 8, DH), f32),
            state, state, state,
            pltpu.VMEM((8, E), bf16),
            pltpu.VMEM((8, 256), f32),
            dma((2,)), dma(()), dma((NSLOT,)), dma((2,)), dma((len(TAIL) - 1,)),
        ],
        compiler_params=pltpu.CompilerParams(vmem_limit_bytes=64 * 2**20, disable_bounds_checks=True),
    )(A_x.reshape(B, D), A_k_cache.reshape(-1, DH), A_v_cache.reshape(-1, DH), A_wq, A_wo.T,
      B_x.reshape(B, D), B_k_cache.reshape(-1, DH), B_v_cache.reshape(-1, DH), B_wq, B_wo.T)
    return out.reshape(B, 1, 2 * D)
```
